```python
import os as _os
_os.environ.setdefault('JAX_PLATFORMS', 'cpu')
import jax
import jax.numpy as jnp

def _softmax(x, axis=-1):
    return jax.nn.softmax(x, axis=axis)

def _gelu(x):
    return jax.nn.gelu(x, approximate=True)

def _silu(x):
    return jax.nn.silu(x)

def _sigmoid(x):
    return jax.nn.sigmoid(x)

def _layernorm(x, axis=-1, eps=1e-05):
    m = jnp.mean(x, axis=axis, keepdims=True)
    v = jnp.var(x, axis=axis, keepdims=True)
    return (x - m) / jnp.sqrt(v + eps)

def _scatter_add(tgt, idx, src, axis=0):
    return tgt.at[idx].add(src)

def _segment_sum(src, seg, n):
    return jax.ops.segment_sum(src, seg, n)

class _Rng:

    def __init__(self, key):
        self._k = key

    def _next(self):
        self._k, sub = jax.random.split(self._k)
        return sub

    def normal(self, shape):
        return jax.random.normal(self._next(), shape, dtype=jnp.bfloat16)

    def randint(self, lo, hi, shape):
        return jax.random.randint(self._next(), shape, lo, hi, dtype=jnp.int32)

    def uniform(self, shape, lo=0.0, hi=1.0):
        return jax.random.uniform(self._next(), shape, jnp.bfloat16, lo, hi)

    def permutation(self, n):
        return jax.random.permutation(self._next(), n)
kernel_name = 'gated_mix__memory_aug_recurrent_mem_tr__glu_gated_geglu__prompt'

def setup_inputs():
    _rng = _Rng(jax.random.key(int.from_bytes(__import__("os").urandom(4), "little")))
    _w = lambda a: (lambda t: t.astype(jnp.bfloat16) if jnp.issubdtype(t.dtype, jnp.floating) else t)(jnp.asarray(a))

    def _A_setup():
        B, S, Dm = (1, 2048, 640)
        H, Dh = (32, 128)
        M, seg = (8, 32)
        seg = min(seg, S)
        S = S // seg * seg
        return {'x': _w((lambda *s: _rng.normal(s) * 0.05)(B, S, Dm)), 'mem0': _w((lambda *s: _rng.normal(s) * 0.4)(B, M, Dm)), 'Wq': _w((lambda *s: _rng.normal(s) * 3.2)(Dm, H, Dh) * Dm ** (-0.5)), 'Wk': _w((lambda *s: _rng.normal(s) * 3.2)(Dm, H, Dh) * Dm ** (-0.5)), 'Wv': _w((lambda *s: _rng.normal(s) * 0.4)(Dm, H, Dh) * Dm ** (-0.5)), 'Wo': _w((lambda *s: _rng.normal(s) * 0.4)(H, Dh, Dm) * (H * Dh) ** (-0.5)), 'seg_len': seg}
    _A_in = _A_setup()

    def _B_setup():
        B, S, Dm, Df = (1, 2048, 640, 1728)
        return {'x': _w((lambda *s: _rng.normal(s) * 0.05)(B, S, Dm)), 'w_gate': _w((lambda *s: _rng.normal(s) * 1.6)(Dm, Df) * Dm ** (-0.5)), 'w_up': _w((lambda *s: _rng.normal(s) * 1.6)(Dm, Df) * Dm ** (-0.5)), 'w_down': _w((lambda *s: _rng.normal(s) * 1.6)(Df, Dm) * Df ** (-0.5))}
    _B_in = _B_setup()
    return {'A_x': _A_in['x'], 'A_mem0': _A_in['mem0'], 'A_Wq': _A_in['Wq'], 'A_Wk': _A_in['Wk'], 'A_Wv': _A_in['Wv'], 'A_Wo': _A_in['Wo'], 'A_seg_len': _A_in['seg_len'], 'B_x': _B_in['x'], 'B_w_gate': _B_in['w_gate'], 'B_w_up': _B_in['w_up'], 'B_w_down': _B_in['w_down'], 'gate_w': _w((lambda *s: _rng.normal(s) * 0.05)(640) * 16.0)}

def reference(A_x, A_mem0, A_Wq, A_Wk, A_Wv, A_Wo, A_seg_len, B_x, B_w_gate, B_w_up, B_w_down, gate_w):

    def _A_ref(x, mem0, Wq, Wk, Wv, Wo, seg_len):
        B, S, Dm = x.shape
        H, Dh = (Wq.shape[1], Wq.shape[2])
        M = mem0.shape[1]
        scale = Dh ** (-0.5)
        n_seg = S // seg_len
        L = M + seg_len
        idx = jnp.arange(L)
        mask = (idx[:, None] < M) | (idx[:, None] >= idx[None, :])
        mem = mem0
        outs = []
        for s in range(n_seg):
            xs = x[:, s * seg_len:(s + 1) * seg_len, :].copy()
            h = jnp.concatenate([mem, xs], axis=1)
            q = jnp.einsum('btd,dhe->bhte', h, Wq)
            k = jnp.einsum('btd,dhe->bhte', h, Wk)
            v = jnp.einsum('btd,dhe->bhte', h, Wv)
            scores = jnp.einsum('bhqe,bhke->bhqk', q, k) * scale
            scores = jnp.where(mask[None, None], scores, -1000000000.0)
            p = _softmax(scores, axis=-1)
            o = jnp.einsum('bhqk,bhke->bhqe', p, v)
            o = jnp.einsum('bhte,hed->btd', o, Wo)
            mem = o[:, :M, :].copy()
            outs.append(o[:, M:, :])
        return jnp.concatenate(outs, axis=1)

    def _B_ref(x, w_gate, w_up, w_down):
        g = jnp.einsum('bsd,df->bsf', x, w_gate)
        u = jnp.einsum('bsd,df->bsf', x, w_up)
        h = _gelu(g) * u
        return jnp.einsum('bsf,fd->bsd', h, w_down)
    x = A_x
    g = _sigmoid((x * gate_w).sum(-1, keepdims=True))
    a = _A_ref(x, A_mem0, A_Wq, A_Wk, A_Wv, A_Wo, A_seg_len)
    b = _B_ref(x, B_w_gate, B_w_up, B_w_down)
    return g * a + (1 - g) * b
```

```python
import functools
import jax
import jax.numpy as jnp
import jax.experimental.pallas as pl
import jax.experimental.pallas.tpu as pltpu

F32 = jnp.float32
BF16 = jnp.bfloat16
U32 = jnp.uint32
NEG = -1000000000.0
TB = (((1,), (1,)), ((), ()))


def _masks():
    qi = jax.lax.broadcasted_iota(jnp.int32, (32, 48), 0)
    kj = jax.lax.broadcasted_iota(jnp.int32, (32, 48), 1)
    existA = kj < 40
    okA = existA & ((qi < 8) | (kj <= qi))
    fillA = jnp.where(existA, NEG, -jnp.inf).astype(F32)
    qi = jax.lax.broadcasted_iota(jnp.int32, (48, 80), 0)
    kj = jax.lax.broadcasted_iota(jnp.int32, (48, 80), 1)
    q_is_mem = (qi >= 16) & (qi < 24)
    q_row = jnp.where(qi < 16, qi + 24, qi + 16)
    q_segB = qi >= 8
    k_is_memA = kj < 8
    k_is_memB = (kj >= 48) & (kj < 56)
    k_row = jnp.where(kj < 48, kj - 8, kj - 16)
    k_segB = kj >= 40
    existB = q_segB == k_segB
    okB = existB & (q_is_mem | k_is_memA | k_is_memB | (k_row <= q_row))
    fillB = jnp.where(existB, NEG, -jnp.inf).astype(F32)
    return okA, fillA, okB, fillB


def _bf(v):
    return pltpu.bitcast(v, BF16)


def _dot(a, b):
    return jnp.dot(a, b, preferred_element_type=F32)


def _dott(a, b):
    return jax.lax.dot_general(a, b, TB, preferred_element_type=F32)


def _glu(g, u):
    return (jax.nn.gelu(g, approximate=True) * u).astype(BF16)


def _kernel(x_hbm, mem0_ref, wq_hbm, wk_hbm, wv_hbm, wo_hbm, wgT_hbm, wuT_hbm, wd_hbm, gw_ref,
            o_ref,
            x_s, mem_ref, stage, wqkv_s, wo_s, gT_s, uT_s, wgu_s, wd_s, b_s, sem_g, sem_f, sem_x,
            *, S, Dm, H, Dh, Df, R0, P1, NIT, GRP, D_S, D_PV, D_WO, CMB):
    i = pl.program_id(0)
    NC = Df // 128
    REM = Df - NC * 128
    assert REM * 2 == 128
    KT = Dm // 128

    def gu_T(Xf, c):
        if c < NC:
            g = _dott(Xf, _bf(gT_s[c * 64:(c + 1) * 64, :]))
            u = _dott(Xf, _bf(uT_s[c * 64:(c + 1) * 64, :]))
        else:
            r = _dott(Xf, _bf(gT_s[NC * 64:(NC + 1) * 64, :]))
            g, u = r[:, :REM], r[:, REM:]
        return _glu(g, u)

    def gu_N(Xf, c):
        if c < NC:
            r = _dot(Xf, _bf(wgu_s[:, c * 256:(c + 1) * 256]))
            g, u = r[:, :128], r[:, 128:]
        else:
            r = _dot(Xf, _bf(wgu_s[:, NC * 256:NC * 256 + 128]))
            g, u = r[:, :REM], r[:, REM:]
        return _glu(g, u)

    def dn(hm, c):
        r0 = c * 64
        r1 = r0 + (64 if c < NC else REM // 2)
        return _dot(hm, _bf(wd_s[r0:r1, :]))

    @pl.when(i == 0)
    def _():
        g32, u32, d32 = wgT_hbm.bitcast(U32), wuT_hbm.bitcast(U32), wd_hbm.bitcast(U32)
        cx0 = pltpu.make_async_copy(x_hbm.at[0:P1], x_s.at[0:P1], sem_x.at[0])
        cx1 = pltpu.make_async_copy(x_hbm.at[P1:R0], x_s.at[P1:R0], sem_x.at[1])
        cx2 = pltpu.make_async_copy(x_hbm.at[R0:S], x_s.at[R0:S], sem_x.at[2])
        cpo = pltpu.make_async_copy(wo_hbm.bitcast(U32), wo_s, sem_x.at[3])
        cx0.start()
        groups = [list(range(c, min(c + GRP, NC + 1))) for c in range(0, NC + 1, GRP)]
        fcps = []
        for gi, grp in enumerate(groups):
            r0 = grp[0] * 64
            r1 = min((grp[-1] + 1) * 64, Df // 2)
            cps = [pltpu.make_async_copy(g32.at[r0:r1], gT_s.at[r0:r1], sem_f.at[gi, 0])]
            ru1 = min(r1, NC * 64)
            if ru1 > r0:
                cps.append(pltpu.make_async_copy(u32.at[r0:ru1], uT_s.at[r0:ru1], sem_f.at[gi, 1]))
            if grp[-1] == NC:
                cps.append(pltpu.make_async_copy(u32.at[NC * 64:Df // 2], gT_s.at[Df // 2:(NC + 1) * 64], sem_f.at[gi, 3]))
            cps.append(pltpu.make_async_copy(d32.at[r0:r1], wd_s.at[r0:r1], sem_f.at[gi, 2]))
            for cp in cps:
                cp.start()
            fcps.append(cps)
        cx1.start()

        def gather(m, par, j):
            w32 = (wq_hbm, wk_hbm, wv_hbm)[m].bitcast(U32)
            return pltpu.make_async_copy(w32.at[:, par, j, :], stage.at[m, par, j], sem_g.at[m, par, j])
        mem_ref[...] = mem0_ref[...]
        ng = len(groups)
        jsplit = [(H // 2) * g // ng for g in range(ng + 1)]

        eye = (jax.lax.broadcasted_iota(jnp.int32, (128, 128), 0)
               == jax.lax.broadcasted_iota(jnp.int32, (128, 128), 1)).astype(BF16)

        def retranspose(src, r0, col0):
            for kt in range(KT):
                t = _dott(eye, _bf(src[r0:r0 + 64, kt * 128:(kt + 1) * 128])).astype(BF16)
                wgu_s[kt * 64:(kt + 1) * 64, col0:col0 + 128] = pltpu.bitcast(t, U32)

        cx0.wait()
        for gi, grp in enumerate(groups):
            for cp in fcps[gi]:
                cp.wait()
            for j in range(jsplit[gi], jsplit[gi + 1]):
                for m in range(3):
                    for par in range(2):
                        gather(m, par, j).start()
            Xf = x_s[0:P1, :]
            hms = [gu_T(Xf, c) for c in grp]
            for c in grp:
                retranspose(gT_s, c * 64, c * 256)
                if c < NC:
                    retranspose(uT_s, c * 64, c * 256 + 128)
            acc = None
            for c, hm in zip(grp, hms):
                d = dn(hm, c)
                acc = d if acc is None else acc + d
            if gi == 0:
                b_s[0:P1, :] = acc
            else:
                b_s[0:P1, :] += acc
        cx1.wait()
        cx2.start()
        cpo.start()

        RB_ = (R0 - P1) // NIT
        JP = (H // 2) // NIT

        def body(r, carry):
            for jj in range(JP):
                j = r * JP + jj
                for m in range(3):
                    gather(m, 0, j).wait()
                    gather(m, 1, j).wait()
            r0 = pl.multiple_of(P1 + r * RB_, 16)
            Xf = x_s[pl.ds(r0, RB_), :]
            units = []
            for jj in range(JP):
                for m in range(3):
                    units.append((jj, m))
            def combine(jj, m):
                j = r * JP + jj
                for d0 in range(0, Dm // 2, 64):
                    a = stage[m, 0, j, d0:d0 + 64, :]
                    b = stage[m, 1, j, d0:d0 + 64, :]
                    wqkv_s[2 * j, d0:d0 + 64, m * Dh:(m + 1) * Dh] = (a & U32(0xFFFF)) | (b << 16)
                    wqkv_s[2 * j + 1, d0:d0 + 64, m * Dh:(m + 1) * Dh] = (a >> 16) | (b & U32(0xFFFF0000))
            acc = None
            hm_prev = None
            for c in range(NC + 2):
                hm = gu_N(Xf, c) if c <= NC else None
                if hm_prev is not None:
                    d = dn(hm_prev, c - 1)
                    acc = d if acc is None else acc + d
                hm_prev = hm
                if units and CMB == 0:
                    combine(*units.pop(0))
            b_s[pl.ds(r0, RB_), :] = acc
            while units:
                combine(*units.pop(0))
            return carry
        jax.lax.fori_loop(0, NIT, body, 0)
        cx2.wait()
        cpo.wait()

    scale = Dh ** (-0.5)
    okA, fillA, okB, fillB = _masks()

    row0 = pl.multiple_of(i * 64, 64)
    X = x_s[pl.ds(row0, 64), :]
    nf = (S - R0) // (S // 64)
    frow0 = pl.multiple_of(R0 + i * nf, nf)
    Xf = x_s[pl.ds(frow0, nf), :]

    ffn_state = {"hm": {}, "acc": None, "next": 0}
    ffn_units = []
    for c in range(NC + 2):
        if c <= NC:
            ffn_units.append(("gu", c))
        if c >= 1:
            ffn_units.append(("dn", c - 1))

    def ffn_run(n):
        for _ in range(n):
            k = ffn_state["next"]
            if k >= len(ffn_units):
                return
            kind, c = ffn_units[k]
            ffn_state["next"] = k + 1
            if kind == "gu":
                ffn_state["hm"][c] = gu_N(Xf, c)
            else:
                d = dn(ffn_state["hm"].pop(c), c)
                ffn_state["acc"] = d if ffn_state["acc"] is None else ffn_state["acc"] + d

    def substep(R, ok, fill, prev, nfill):
        qkv, pe, ov = {}, {}, {}
        saved = []
        acc = None
        T = H + D_WO
        for t in range(T):
            if t < H:
                r = _dot(R, _bf(wqkv_s[t])).astype(BF16)
                q, k, v = r[:, 0:Dh], r[:, Dh:2 * Dh], r[:, 2 * Dh:3 * Dh]
                if prev is None:
                    saved.append((q[32:48], k, v))
                    q = q[0:32]
                else:
                    pq, pk, pv = prev[t]
                    q = jnp.concatenate([pq, q], axis=0)
                    k = jnp.concatenate([pk, k], axis=0)
                    v = jnp.concatenate([pv, v], axis=0)
                qkv[t] = (q, k, v)
            else:
                ffn_run(nfill[t - H])
            h = t - D_S
            if 0 <= h < H:
                q, k, v = qkv[h]
                s = _dott(q, k)
                s = jnp.where(ok, s * scale, fill)
                m = jnp.max(s, axis=-1, keepdims=True)
                p = jnp.exp(s - m)
                l = jnp.sum(p, axis=-1, keepdims=True)
                pe[h] = (p.astype(BF16), l)
            h = t - D_PV
            if 0 <= h < H:
                p, l = pe.pop(h)
                o = _dot(p, qkv.pop(h)[2])
                ov[h] = (o / l).astype(BF16)
            h = t - D_WO
            if 0 <= h < H:
                d = _dot(ov.pop(h), _bf(wo_s[h * Dh // 2:(h + 1) * Dh // 2, :]))
                acc = d if acc is None else acc + d
        ffn_run(nfill[-1])
        return acc, saved

    nu = len(ffn_units)
    half = nu // 2

    def split(n, parts):
        base = [n // parts] * parts
        for k in range(n % parts):
            base[k] += 1
        return base

    mem = mem_ref[...]
    RA = jnp.concatenate([mem, X[0:40]], axis=0)
    accA, saved = substep(RA, okA, fillA, None, split(half, D_WO + 1))
    memB = accA[0:8].astype(BF16)
    RB = jnp.concatenate([memB, X[40:64]], axis=0)
    accB, _ = substep(RB, okB, fillB, saved, split(nu - half, D_WO + 1))
    mem_ref[...] = accB[16:24].astype(BF16)
    ffn_run(nu)
    b_s[pl.ds(frow0, nf), :] = ffn_state["acc"]

    a = jnp.concatenate([accA[8:32], accB[0:16], accB[24:48]], axis=0)
    b = b_s[pl.ds(row0, 64), :]
    gate = jax.nn.sigmoid(jnp.sum(X.astype(F32) * gw_ref[...].astype(F32), axis=-1, keepdims=True))
    o_ref[...] = (gate * a + (1.0 - gate) * b).astype(o_ref.dtype)


@jax.jit
def _run(A_x, A_mem0, A_Wq, A_Wk, A_Wv, A_Wo, B_w_gate, B_w_up, B_w_down, gate_w):
    D_S, D_PV, D_WO, P1, NIT, GRP, CMB = 1, 3, 4, 256, 4, 2, 1
    B, S, Dm = A_x.shape
    H, Dh = A_Wq.shape[1], A_Wq.shape[2]
    M = A_mem0.shape[1]
    Df = B_w_gate.shape[1]
    assert B == 1 and M == 8 and S % 128 == 0
    R0 = S // 2
    NC = Df // 128
    x = A_x.reshape(S, Dm)
    mem0 = A_mem0.reshape(M, Dm)
    wq = A_Wq.reshape(Dm // 2, 2, H, Dh)
    wk = A_Wk.reshape(Dm // 2, 2, H, Dh)
    wv = A_Wv.reshape(Dm // 2, 2, H, Dh)
    wo = A_Wo.reshape(H * Dh, Dm)
    gw = gate_w.reshape(1, Dm)
    hbm = pl.BlockSpec(memory_space=pltpu.HBM)
    full = lambda shp: pl.BlockSpec(shp, lambda i: (0,) * len(shp))
    ngrp = -(-(NC + 1) // GRP)
    out = pl.pallas_call(
        functools.partial(_kernel, S=S, Dm=Dm, H=H, Dh=Dh, Df=Df, R0=R0, P1=P1, NIT=NIT, GRP=GRP,
                          D_S=D_S, D_PV=D_PV, D_WO=D_WO, CMB=CMB),
        grid=(S // 64,),
        in_specs=[hbm, full((M, Dm)), hbm, hbm, hbm, hbm, hbm, hbm, hbm, full((1, Dm))],
        out_specs=pl.BlockSpec((64, Dm), lambda i: (i, 0)),
        out_shape=jax.ShapeDtypeStruct((S, Dm), A_x.dtype),
        scratch_shapes=[
            pltpu.VMEM((S, Dm), BF16),
            pltpu.VMEM((M, Dm), BF16),
            pltpu.VMEM((3, 2, H // 2, Dm // 2, Dh), U32),
            pltpu.VMEM((H, Dm // 2, 3 * Dh), U32),
            pltpu.VMEM((H * Dh // 2, Dm), U32),
            pltpu.VMEM(((NC + 1) * 64, Dm), U32),
            pltpu.VMEM((NC * 64, Dm), U32),
            pltpu.VMEM((Dm // 2, NC * 256 + 128), U32),
            pltpu.VMEM((Df // 2, Dm), U32),
            pltpu.VMEM((S, Dm), F32),
            pltpu.SemaphoreType.DMA((3, 2, H // 2)),
            pltpu.SemaphoreType.DMA((ngrp, 4)),
            pltpu.SemaphoreType.DMA((4,)),
        ],
        compiler_params=pltpu.CompilerParams(dimension_semantics=("arbitrary",),
                                             vmem_limit_bytes=100 * 1024 * 1024),
    )(x, mem0, wq, wk, wv, wo, B_w_gate.T, B_w_up.T, B_w_down, gw)
    return out.reshape(B, S, Dm)


def pallas_gated_mix__memory_aug_recurrent_mem_tr__glu_gated_geglu__prompt_kernel(
    A_x, A_mem0, A_Wq, A_Wk, A_Wv, A_Wo, A_seg_len, B_x, B_w_gate, B_w_up, B_w_down, gate_w,
):
    if isinstance(A_seg_len, int):
        assert A_seg_len == 32
    return _run(A_x, A_mem0, A_Wq, A_Wk, A_Wv, A_Wo, B_w_gate, B_w_up, B_w_down, gate_w)
```

```python
import functools

import jax
import jax.numpy as jnp
import jax.experimental.pallas as pl
import jax.experimental.pallas.tpu as pltpu

F32 = jnp.float32
BF16 = jnp.bfloat16
U32 = jnp.uint32
NEG = -1000000000.0
TB = (((1,), (1,)), ((), ()))

L1, L2, L3, L4, LV = 270, 340, 230, 140, 160
VL = 1
PRE = (0, 1, 0, 3)
HOLD = 1
LAG = 4
UNR = 2
NXP = 4
RBLK = 128
NG = 4
W0 = 256
GR = 64


def _masks():
    qi = jax.lax.broadcasted_iota(jnp.int32, (32, 48), 0)
    kj = jax.lax.broadcasted_iota(jnp.int32, (32, 48), 1)
    existA = kj < 40
    okA = existA & ((qi < 8) | (kj <= qi))
    fillA = jnp.where(existA, NEG, -jnp.inf).astype(F32)
    qi = jax.lax.broadcasted_iota(jnp.int32, (48, 80), 0)
    kj = jax.lax.broadcasted_iota(jnp.int32, (48, 80), 1)
    q_is_mem = qi < 8
    q_row = jnp.where(qi < 32, qi + 32, qi - 8)
    q_segB = (qi < 32) | (qi >= 40)
    k_is_memA = kj < 8
    k_is_memB = (kj >= 48) & (kj < 56)
    k_row = jnp.where(kj < 48, kj - 8, kj - 16)
    k_segB = kj >= 40
    existB = q_segB == k_segB
    okB = existB & (q_is_mem | k_is_memA | k_is_memB | (k_row <= q_row))
    fillB = jnp.where(existB, NEG, -jnp.inf).astype(F32)
    return okA, fillA, okB, fillB


def _bf(v):
    return pltpu.bitcast(v, BF16)


def _dot(a, b):
    return jnp.dot(a, b, preferred_element_type=F32)


def _dott(a, b):
    return jax.lax.dot_general(a, b, TB, preferred_element_type=F32)


def _glu(g, u):
    return (jax.nn.gelu(g, approximate=True) * u).astype(BF16)


def _gate(x, gw):
    z = jnp.sum(x.astype(F32) * gw, axis=-1, keepdims=True)
    return 0.5 * jnp.tanh(0.5 * z) + 0.5


def _kernel(x_hbm, mem0_hbm, wq_hbm, wk_hbm, wv_hbm, wo_hbm, wgT_hbm, wuT_hbm, wd_hbm, gw_hbm,
            o_hbm,
            x_s, mem_ref, stage, wqkv_s, wo_s, gT_s, uT_s, wgu_s, wd_s, b_s, o_s, gw_s, gate_s, sems,
            *, S, Dm, H, Dh, Df):
    R0 = S // 2
    NIT = S // 64 // UNR
    NC = Df // 128
    REM = Df - NC * 128
    assert REM * 2 == 128 and (NC - 1) % 2 == 0
    KT = Dm // 128
    NPAIR = (NC - 1) // 2
    JP = (H // 2) // NG
    SEM_W, SEM_X, SEM_F, SEM_G = 0, 4, 4 + NXP, 4 + NXP + NPAIR
    SEM_O = SEM_G + NG
    SEM_OUT = SEM_O + 1
    SEM_M = SEM_O + 2

    g32, u32, d32 = wgT_hbm.bitcast(U32), wuT_hbm.bitcast(U32), wd_hbm.bitcast(U32)
    XP_ = (S - W0) // NXP
    PB = XP_ // 4
    assert PB % 16 == 0
    RN = NC * 64
    cw = [[pltpu.make_async_copy(g32.at[RN:Df // 2], gT_s.at[RN:Df // 2], sems.at[SEM_W]),
           pltpu.make_async_copy(u32.at[RN:Df // 2], gT_s.at[Df // 2:RN + 64], sems.at[SEM_W]),
           pltpu.make_async_copy(x_hbm.at[0:128], x_s.at[0:128], sems.at[SEM_W])],
          [pltpu.make_async_copy(g32.at[0:64], gT_s.at[0:64], sems.at[SEM_W + 1]),
           pltpu.make_async_copy(u32.at[0:64], uT_s.at[0:64], sems.at[SEM_W + 1])],
          [pltpu.make_async_copy(x_hbm.at[128:W0], x_s.at[128:W0], sems.at[SEM_W + 2])],
          [pltpu.make_async_copy(d32.at[RN:Df // 2], wd_s.at[RN:Df // 2], sems.at[SEM_W + 3]),
           pltpu.make_async_copy(d32.at[0:64], wd_s.at[0:64], sems.at[SEM_W + 3])]]
    cm = [pltpu.make_async_copy(mem0_hbm, mem_ref, sems.at[SEM_M]),
          pltpu.make_async_copy(gw_hbm, gw_s, sems.at[SEM_M])]

    def cx(p):
        r = pl.ds(pl.multiple_of(W0 + p * XP_, 16), XP_)
        return pltpu.make_async_copy(x_hbm.at[r], x_s.at[r], sems.at[SEM_X + p])

    def cf(k):
        r = pl.ds(pl.multiple_of(64 + k * 128, 64), 128)
        return [pltpu.make_async_copy(src.at[r], dst.at[r], sems.at[SEM_F + k])
                for src, dst in ((g32, gT_s), (u32, uT_s), (d32, wd_s))]

    def gather(g, jj, m, par):
        w32 = (wq_hbm, wk_hbm, wv_hbm)[m].bitcast(U32)
        return pltpu.make_async_copy(w32.at[:, par, g * JP + jj, :], stage.at[g, jj, m, par], sems.at[SEM_G + g])

    def start_gathers(g):
        for jj in range(JP):
            for m in range(3):
                for par in range(2):
                    gather(g, jj, m, par).start()

    cpo = pltpu.make_async_copy(wo_hbm.bitcast(U32), wo_s, sems.at[SEM_O])

    def gu_rem(Xf):
        r = _dott(Xf, _bf(gT_s[RN:RN + 64, :]))
        return _glu(r[:, :REM], r[:, REM:])

    def gu_0(Xf):
        return _glu(_dott(Xf, _bf(gT_s[0:64, :])), _dott(Xf, _bf(uT_s[0:64, :])))

    def dn_first(h_rem, h0):
        return _dot(h_rem, _bf(wd_s[RN:Df // 2, :])) + _dot(h0, _bf(wd_s[0:64, :]))

    for cp in cw[0] + cw[1]:
        cp.start()
    for cp in cw[2] + cw[3]:
        cp.start()
    for cp in cw[0]:
        cp.wait()
    for p in range(NXP):
        cx(p).start()
    ha_rem = gu_rem(x_s[0:128, :])
    for cp in cw[1]:
        cp.wait()
    for cp in cm:
        cp.start()
    for k in range(NPAIR):
        for cp in cf(k):
            cp.start()
    ha0 = gu_0(x_s[0:128, :])
    for cp in cw[2]:
        cp.wait()
    hb_rem = gu_rem(x_s[128:W0, :])
    hb0 = gu_0(x_s[128:W0, :])
    for cp in cw[3]:
        cp.wait()
    b_s[0:128, :] = dn_first(ha_rem, ha0)
    b_s[128:W0, :] = dn_first(hb_rem, hb0)

    def peel(p, carry):
        cx(p).wait()
        nb = XP_ // PB
        hms = {}
        for rb in range(nb + 1):
            if rb < nb:
                Xf = x_s[pl.ds(pl.multiple_of(W0 + p * XP_ + rb * PB, 16), PB), :]
                hms[rb] = (gu_rem(Xf), gu_0(Xf))
            if rb >= 1:
                b_s[pl.ds(pl.multiple_of(W0 + p * XP_ + (rb - 1) * PB, 16), PB), :] = dn_first(*hms.pop(rb - 1))
        return carry
    jax.lax.fori_loop(0, NXP, peel, 0)
    start_gathers(0)
    start_gathers(1)
    for cp in cm:
        cp.wait()

    def pair_body(k, g):
        for cp in cf(k):
            cp.wait()
        if g is not None:
            pltpu.make_async_copy(stage.at[g], stage.at[g], sems.at[SEM_G + g]).wait()

            @pl.when(g == 0)
            def _():
                cpo.start()
        w0 = pl.multiple_of(64 + k * 128, 64)
        nb = R0 // RBLK

        def tr(cc, which, kt):
            src = (gT_s, uT_s)[which]
            t = _bf(src[pl.ds(w0 + cc * 64, 64), kt * 128:(kt + 1) * 128]).T
            wgu_s[2 * k + cc, kt * 64:(kt + 1) * 64, which * 128:(which + 1) * 128] = pltpu.bitcast(t, U32)

        def comb(jj, m, d0):
            j = g * JP + jj
            a = stage[g, jj, m, 0, d0:d0 + 64, :]
            b = stage[g, jj, m, 1, d0:d0 + 64, :]
            wqkv_s[2 * j, d0:d0 + 64, m * Dh:(m + 1) * Dh] = (a & U32(0xFFFF)) | (b << 16)
            wqkv_s[2 * j + 1, d0:d0 + 64, m * Dh:(m + 1) * Dh] = (a >> 16) | (b & U32(0xFFFF0000))

        trs = [functools.partial(tr, cc, which, kt) for cc in range(2) for which in range(2) for kt in range(KT)]
        GN = S // (NPAIR - NG)
        gvals = {}

        def gate_rows(n):
            if n < GN // GR:
                r = pl.ds(pl.multiple_of(k * GN + n * GR, GR), GR)
                gw = gw_s[...].astype(F32).reshape(1, Dm)
                gvals[n] = jnp.broadcast_to(_gate(x_s[r, :], gw), (GR, 128))
            if n >= 1:
                r = pl.ds(pl.multiple_of(k * GN + (n - 1) * GR, GR), GR)
                gate_s[r, :] = gvals.pop(n - 1)

        if g is None:
            cbs = [functools.partial(gate_rows, n) for n in range(GN // GR + 1)]
        else:
            cbs = [functools.partial(comb, jj, m, d0) for jj in range(JP) for m in range(3)
                   for d0 in range(0, Dm // 2, 64)]
        nslot = 3 * nb - 1
        slots = [[] for _ in range(nslot)]
        for n, f in enumerate(trs):
            slots[n * nslot // len(trs)].append(f)
        for n, f in enumerate(cbs):
            slots[n * nslot // len(cbs)].append(f)

        def side_run():
            if slots:
                for f in slots.pop(0):
                    f()
        hms = {}
        for rb in range(nb + 1):
            if rb < nb:
                Xf = x_s[rb * RBLK:(rb + 1) * RBLK, :]
                gg = _dott(Xf, _bf(gT_s[pl.ds(w0, 128), :]))
                side_run()
                uu = _dott(Xf, _bf(uT_s[pl.ds(w0, 128), :]))
                side_run()
                hms[rb] = _glu(gg, uu)
            if rb >= 1:
                b_s[(rb - 1) * RBLK:rb * RBLK, :] += _dot(hms.pop(rb - 1), _bf(wd_s[pl.ds(w0, 128), :]))
                side_run()
        assert not slots

    def loop1(k, carry):
        pair_body(k, None)
        return carry
    jax.lax.fori_loop(0, NPAIR - NG, loop1, 0)
    start_gathers(2)
    start_gathers(3)

    def loop2(g, carry):
        pair_body(g + (NPAIR - NG), g)
        return carry
    jax.lax.fori_loop(0, NG, loop2, 0)
    cpo.wait()

    def emit(p, a):
        r = pl.ds(pl.multiple_of(p * 64, 64), 64)
        gate = jnp.concatenate([gate_s[r, :]] * KT, axis=1)
        o_s[r, :] = (gate * a + (1.0 - gate) * b_s[r, :]).astype(o_s.dtype)

    def out_copy(p, n):
        r = pl.ds(pl.multiple_of(p * 64, 64), 64 * n)
        return pltpu.make_async_copy(o_s.at[r], o_hbm.at[r], sems.at[SEM_OUT])

    scale = Dh ** (-0.5)
    nf = (S - R0) // (S // 64)

    def main(it, carry):
        okA, fillA, okB, fillB = _masks()

        def make_ffn(p):
            frow = pl.ds(pl.multiple_of(R0 + p * nf, nf), nf)
            Xf = x_s[frow, :]
            st = {"hm": {}, "acc": b_s[frow, :]}
            units = []

            def gu(c):
                r = _dot(Xf, _bf(wgu_s[c]))
                st["hm"][c] = _glu(r[:, :128], r[:, 128:])
                return 80

            def dn(c):
                st["acc"] = st["acc"] + _dot(st["hm"].pop(c), _bf(wd_s[(c + 1) * 64:(c + 2) * 64, :]))
                if c == NC - 2:
                    b_s[frow, :] = st["acc"]
                return 40
            for k in range(NC - 1 + LAG):
                if k < NC - 1:
                    units.append(functools.partial(gu, k))
                if k >= LAG:
                    units.append(functools.partial(dn, k - LAG))
            return units

        ffn_units = []

        def substep(R, ok, fill, prev, pre, last):
            nq, na = (3, 2) if prev is None else (2, 3)
            dA, dW = na * 4 + 4, 5 * na * 4
            pe, ov, saved, proj = {}, {}, {}, {}
            st = {"acc": None}
            Rq, Rkv = (R[0:32], R) if prev is None else (R, R[0:32])

            def doProj(kind, h):
                c = {"q": 0, "k": 1, "v": 2}[kind]
                r = _dot(Rq if kind == "q" else Rkv, _bf(wqkv_s[h, :, c * Dh:(c + 1) * Dh])).astype(BF16)
                if kind != "q":
                    if prev is None:
                        saved[(kind, h)] = r
                    else:
                        r = jnp.concatenate([prev[(kind, h)], r], axis=0)
                proj[(kind, h)] = r

            def doS(h):
                s = _dott(proj.pop(("q", h)), proj.pop(("k", h)))
                s = jnp.where(ok, s * scale, fill)
                m = jnp.max(s, axis=-1, keepdims=True)
                p = jnp.exp(s - m)
                l = jnp.sum(p, axis=-1, keepdims=True)
                pe[h] = (p.astype(BF16), l)

            def doP(h):
                p, l = pe.pop(h)
                o = _dot(p, proj.pop(("v", h)))
                ov[h] = (o / l).astype(BF16)

            def doW(h):
                d = _dot(ov.pop(h), _bf(wo_s[h * Dh // 2:(h + 1) * Dh // 2, :]))
                st["acc"] = d if st["acc"] is None else st["acc"] + d

            stream = []
            for h in range(H + VL):
                if h < H:
                    stream += [("k", h), ("q", h)]
                if h >= VL:
                    stream.append(("v", h - VL))
            t = 0
            nS = nP = nW = 0
            rS, rP, rW, rV = {}, {}, {}, {}
            while nW < H:
                hold = last and len(stream) <= 3 * HOLD
                if nS in rS and rS[nS] <= t:
                    doS(nS)
                    rP[nS] = t + L2
                    t += dA
                    nS += 1
                elif nP < nS and nP in rV and max(rP[nP], rV[nP]) <= t:
                    doP(nP)
                    rW[nP] = t + L3
                    t += dA
                    nP += 1
                elif last and not stream and ffn_units:
                    t += ffn_units.pop(0)()
                elif nW < nP and rW[nW] <= t and not (hold and stream):
                    doW(nW)
                    t += dW
                    nW += 1
                elif stream:
                    kind, h = stream.pop(0)
                    doProj(kind, h)
                    t += 5 * (na if kind == "q" else nq) * 4
                    if kind == "q":
                        rS[h] = t + L1
                        if pre > 0 and ffn_units:
                            t += ffn_units.pop(0)()
                            pre -= 1
                    elif kind == "v":
                        rV[h] = t + LV
                elif ffn_units:
                    t += ffn_units.pop(0)()
                else:
                    t += 8
            tend = t + L4
            while ffn_units and (last or t < tend):
                t += ffn_units.pop(0)()
            return st["acc"], saved

        mem = mem_ref[...]
        for u in range(UNR):
            ffn_units.extend(make_ffn(it * UNR + u))
        for u in range(UNR):
            p = it * UNR + u
            X = x_s[pl.ds(pl.multiple_of(p * 64, 64), 64), :]
            RA = jnp.concatenate([mem, X[0:40]], axis=0)
            accA, saved = substep(RA, okA, fillA, None, PRE[2 * u], False)
            memB = accA[0:8].astype(BF16)
            RB = jnp.concatenate([memB, X[40:64], X[24:40]], axis=0)
            accB, _ = substep(RB, okB, fillB, saved, PRE[2 * u + 1], u == UNR - 1)
            mem = accB[0:8].astype(BF16)
            emit(p, jnp.concatenate([accA[8:32], accB[32:48], accB[8:32]], axis=0))
        assert not ffn_units
        mem_ref[...] = mem
        out_copy(it * UNR, UNR).start()
        return carry

    jax.lax.fori_loop(0, NIT, main, 0)
    out_copy(0, NIT * UNR).wait()


@jax.jit
def _run(A_x, A_mem0, A_Wq, A_Wk, A_Wv, A_Wo, B_w_gate, B_w_up, B_w_down, gate_w):
    B, S, Dm = A_x.shape
    H, Dh = A_Wq.shape[1], A_Wq.shape[2]
    M = A_mem0.shape[1]
    Df = B_w_gate.shape[1]
    assert B == 1 and M == 8 and S % 128 == 0
    NC = Df // 128
    hbm = pl.BlockSpec(memory_space=pltpu.HBM)
    nsem = 4 + NXP + (NC - 1) // 2 + NG + 3
    out = pl.pallas_call(
        functools.partial(_kernel, S=S, Dm=Dm, H=H, Dh=Dh, Df=Df),
        in_specs=[hbm] * 10,
        out_specs=hbm,
        out_shape=jax.ShapeDtypeStruct((S, Dm), A_x.dtype),
        scratch_shapes=[
            pltpu.VMEM((S, Dm), BF16),
            pltpu.VMEM((M, Dm), BF16),
            pltpu.VMEM((NG, H // 2 // NG, 3, 2, Dm // 2, Dh), U32),
            pltpu.VMEM((H, Dm // 2, 3 * Dh), U32),
            pltpu.VMEM((H * Dh // 2, Dm), U32),
            pltpu.VMEM(((NC + 1) * 64, Dm), U32),
            pltpu.VMEM((NC * 64, Dm), U32),
            pltpu.VMEM((NC - 1, Dm // 2, 256), U32),
            pltpu.VMEM((Df // 2, Dm), U32),
            pltpu.VMEM((S, Dm), F32),
            pltpu.VMEM((S, Dm), BF16),
            pltpu.VMEM((Dm,), BF16),
            pltpu.VMEM((S, 128), F32),
            pltpu.SemaphoreType.DMA((nsem,)),
        ],
        compiler_params=pltpu.CompilerParams(vmem_limit_bytes=100 * 1024 * 1024),
    )(A_x.reshape(S, Dm), A_mem0.reshape(M, Dm),
      A_Wq.reshape(Dm // 2, 2, H, Dh), A_Wk.reshape(Dm // 2, 2, H, Dh), A_Wv.reshape(Dm // 2, 2, H, Dh),
      A_Wo.reshape(H * Dh, Dm), B_w_gate.T, B_w_up.T, B_w_down, gate_w)
    return out.reshape(B, S, Dm)


def pallas_gated_mix__memory_aug_recurrent_mem_tr__glu_gated_geglu__prompt_kernel(
    A_x, A_mem0, A_Wq, A_Wk, A_Wv, A_Wo, A_seg_len, B_x, B_w_gate, B_w_up, B_w_down, gate_w,
):
    if isinstance(A_seg_len, int):
        assert A_seg_len == 32
    return _run(A_x, A_mem0, A_Wq, A_Wk, A_Wv, A_Wo, B_w_gate, B_w_up, B_w_down, gate_w)
```
